```python
import os as _os
_os.environ.setdefault("JAX_PLATFORMS", "cpu")
import jax
import jax.numpy as jnp

def _softmax(x, axis=-1):
    return jax.nn.softmax(x, axis=axis)
def _gelu(x):
    return jax.nn.gelu(x, approximate=True)
def _silu(x):
    return jax.nn.silu(x)
def _sigmoid(x):
    return jax.nn.sigmoid(x)
def _layernorm(x, axis=-1, eps=1e-5):
    m = jnp.mean(x, axis=axis, keepdims=True)
    v = jnp.var(x, axis=axis, keepdims=True)
    return (x - m) / jnp.sqrt(v + eps)
def _scatter_add(tgt, idx, src, axis=0):
    return tgt.at[idx].add(src)
def _segment_sum(src, seg, n):
    return jax.ops.segment_sum(src, seg, n)
class _Rng:
    def __init__(self, key):
        self._k = key
    def _next(self):
        self._k, sub = jax.random.split(self._k)
        return sub
    def normal(self, shape):
        return jax.random.normal(self._next(), shape, dtype=jnp.bfloat16)
    def randint(self, lo, hi, shape):
        return jax.random.randint(self._next(), shape, lo, hi, dtype=jnp.int32)
    def uniform(self, shape, lo=0.0, hi=1.0):
        return jax.random.uniform(self._next(), shape, jnp.bfloat16, lo, hi)
    def permutation(self, n):
        return jax.random.permutation(self._next(), n)


kernel_name = 'gated_mix__ssm_conv_s5__glu_gated_geglu__prompt'

def setup_inputs():
    _rng = _Rng(jax.random.key(int.from_bytes(__import__("os").urandom(4), "little")))
    _w = (lambda a: (lambda t: t.astype(jnp.bfloat16) if jnp.issubdtype(t.dtype, jnp.floating) else t)(jnp.asarray(a)))
    def _A_setup():
        B, S, D = 1, 2048, 1024
        P = D
        Lambda_re = -0.5 * jnp.exp((lambda *s: _rng.normal(s) * 0.4)(P))
        Lambda_im = (lambda *s: _rng.normal(s) * 0.4)(P) * 1.0
        B_re = (lambda *s: _rng.normal(s) * 0.4)(P, D) * (D ** -0.5)
        B_im = (lambda *s: _rng.normal(s) * 0.4)(P, D) * (D ** -0.5)
        C_re = (lambda *s: _rng.normal(s) * 0.4)(D, P) * (P ** -0.5)
        C_im = (lambda *s: _rng.normal(s) * 0.4)(D, P) * (P ** -0.5)
        log_dt = (lambda *s: _rng.normal(s) * 0.4)(P) * 0.3 - 2.0
        Dskip = (lambda *s: _rng.normal(s) * 0.4)(D)
        return {
            "x": _w((lambda *s: _rng.normal(s) * 0.05)(B, S, D)),
            "Lambda_re": _w(Lambda_re),
            "Lambda_im": _w(Lambda_im),
            "B_re": _w(B_re),
            "B_im": _w(B_im),
            "C_re": _w(C_re),
            "C_im": _w(C_im),
            "log_dt": _w(log_dt),
            "Dskip": _w(Dskip),
        }
    _A_in = _A_setup()

    def _B_setup():
        B, S, Dm, Df = 1, 2048, 1024, 3584
        return {
            "x": _w((lambda *s: _rng.normal(s) * 0.05)(B, S, Dm)),
            "w_gate": _w((lambda *s: _rng.normal(s) * 1.6)(Dm, Df) * (Dm ** -0.5)),
            "w_up": _w((lambda *s: _rng.normal(s) * 1.6)(Dm, Df) * (Dm ** -0.5)),
            "w_down": _w((lambda *s: _rng.normal(s) * 1.6)(Df, Dm) * (Df ** -0.5)),
        }
    _B_in = _B_setup()

    return {
        "A_x": _A_in["x"],
        "A_Lambda_re": _A_in["Lambda_re"],
        "A_Lambda_im": _A_in["Lambda_im"],
        "A_B_re": _A_in["B_re"],
        "A_B_im": _A_in["B_im"],
        "A_C_re": _A_in["C_re"],
        "A_C_im": _A_in["C_im"],
        "A_log_dt": _A_in["log_dt"],
        "A_Dskip": _A_in["Dskip"],
        "B_x": _B_in["x"],
        "B_w_gate": _B_in["w_gate"],
        "B_w_up": _B_in["w_up"],
        "B_w_down": _B_in["w_down"],
        "gate_w": _w((lambda *s: _rng.normal(s) * 0.05)(1024) * 16.0),
    }

def reference(A_x, A_Lambda_re, A_Lambda_im, A_B_re, A_B_im, A_C_re, A_C_im, A_log_dt, A_Dskip, B_x, B_w_gate, B_w_up, B_w_down, gate_w):
    def _A_ref(x, Lambda_re, Lambda_im, B_re, B_im, C_re, C_im, log_dt, Dskip):
        Bsz, L, H = x.shape
        Lam = Lambda_re + 1j * Lambda_im
        Bmat = B_re + 1j * B_im
        Cmat = C_re + 1j * C_im
        dt = jnp.exp(log_dt)
        Lam_bar = jnp.exp(dt * Lam)
        B_bar = ((Lam_bar - 1.0) / Lam)[:, None] * Bmat
        Bu = jnp.einsum("bld,pd->blp", x + 0j, B_bar)
        h = jnp.zeros_like(Bu[:, 0, :])
        hs = []
        for t in range(L):
            h = Lam_bar[None, :] * h + Bu[:, t, :]
            hs.append(h)
        hseq = jnp.stack(hs, 1)
        y = 2.0 * jnp.einsum("blp,dp->bld", hseq, Cmat).real + x * Dskip[None, None, :]
        return y

    def _B_ref(x, w_gate, w_up, w_down):
        g = jnp.einsum("bsd,df->bsf", x, w_gate)
        u = jnp.einsum("bsd,df->bsf", x, w_up)
        h = _gelu(g) * u
        return jnp.einsum("bsf,fd->bsd", h, w_down)

    x = A_x
    g = _sigmoid((x * gate_w).sum(-1, keepdims=True))
    a = _A_ref(x, A_Lambda_re, A_Lambda_im, A_B_re, A_B_im, A_C_re, A_C_im, A_log_dt, A_Dskip)
    b = _B_ref(x, B_w_gate, B_w_up, B_w_down)
    return g * a + (1 - g) * b
```

```python
import functools
import numpy as np
import jax
import jax.numpy as jnp
from jax import lax
from jax.experimental import pallas as pl
from jax.experimental.pallas import tpu as pltpu

F32 = jnp.float32
BF16 = jnp.bfloat16
U32 = jnp.uint32
LANES = 128
SUB = 8

def _dot(a, b):
    return jnp.dot(a, b, preferred_element_type=F32)

def _dot_t(a, b):
    return lax.dot_general(a, b, (((1,), (1,)), ((), ())), preferred_element_type=F32)

def _pk(v):
    return pltpu.bitcast(v.astype(BF16), U32)

def _bf(u):
    return pltpu.bitcast(u, BF16)

def _cmul(ar, ai, br, bi):
    return ar * br - ai * bi, ar * bi + ai * br

def lcomb(a11, a12, a21, a22):
    return [a11 + a22, a21 + a22, a11, a22, a11 + a12, a21 - a11, a12 - a22]

def rcomb(b11, b12, b21, b22):
    return [b11 + b22, b11, b12 - b22, b21 - b11, b22, b11 + b12, b21 + b22]

def comb2(comb, g):
    out = [None] * 49
    outer = {}
    for i in range(2):
        for k in range(2):
            outer[i, k] = comb(g[i][k], g[i][2 + k], g[2 + i][k], g[2 + i][2 + k])
    for n in range(7):
        inner = comb(outer[0, 0][n], outer[0, 1][n], outer[1, 0][n], outer[1, 1][n])
        for m in range(7):
            out[n * 7 + m] = inner[m]
    return out

def zero_of(v):
    return (lax.bitcast_convert_type(v, U32) >> 16) >> 16

def rcomb2_packed(load, store, dep=None, ndeps=None):
    if SKIP[0]:
        return
    raw = [[load(r, c) for c in range(4)] for r in range(4)]
    if dep is not None:
        raw = [[v | dep for v in row] for row in raw]
    passthrough = {8: (0, 0), 11: (1, 1), 29: (2, 2), 32: (3, 3)}
    if ORDER[0] == 0:
        halves = []
        for e in range(2):
            g = [[pltpu.unpack_elementwise(raw[r][c], index=e, packed_dtype=BF16, unpacked_dtype=F32)
                  for c in range(4)] for r in range(4)]
            halves.append(comb2(rcomb, g))
        for nm in range(49):
            if nm in passthrough:
                r, c = passthrough[nm]
                store(nm, raw[r][c])
            else:
                store(nm, pltpu.pack_elementwise([halves[0][nm], halves[1][nm]], packed_dtype=BF16))
    else:
        cache = {}
        def un(r, c, e):
            if ORDER[0] == 2 and (r, c, e) in cache:
                return cache[r, c, e]
            v = pltpu.unpack_elementwise(raw[r][c], index=e, packed_dtype=BF16, unpacked_dtype=F32)
            cache[r, c, e] = v
            return v
        terms = [((0, 0), (1, 1), 1), ((0, 0), None, 0), ((0, 1), (1, 1), -1), ((1, 0), (0, 0), -1),
                 ((1, 1), None, 0), ((0, 0), (0, 1), 1), ((1, 0), (1, 1), 1)]
        for n, (ta, tb, sg) in enumerate(terms):
            inner = []
            for e in range(2):
                o = []
                for i in range(2):
                    for k in range(2):
                        a = un(2 * ta[0] + i, 2 * ta[1] + k, e)
                        if tb is not None:
                            b = un(2 * tb[0] + i, 2 * tb[1] + k, e)
                            a = a + b if sg > 0 else a - b
                        if ndeps is not None and n > 0:
                            a = lax.bitcast_convert_type(lax.bitcast_convert_type(a, U32) | ndeps[n], F32)
                        o.append(a)
                inner.append(rcomb(*o))
            for m in range(7):
                nm = n * 7 + m
                if nm in passthrough:
                    r, c = passthrough[nm]
                    store(nm, raw[r][c])
                else:
                    store(nm, pltpu.pack_elementwise([inner[0][m], inner[1][m]], packed_dtype=BF16))

ORDER = [0]
SKIP = [0]

def strassen_out(prod):
    add = lambda a, b: jax.tree.map(lambda p, q: p + q, a, b)
    sub = lambda a, b: jax.tree.map(lambda p, q: p - q, a, b)
    m5 = prod(4); m3 = prod(2); c12 = add(m3, m5)
    m4 = prod(3); m2 = prod(1); c21 = add(m2, m4)
    t = sub(m4, m5); u = sub(m3, m2)
    m1 = prod(0); t = add(t, m1); u = add(u, m1)
    c11 = add(t, prod(6))
    c22 = add(u, prod(5))
    return [c11, c12, c21, c22]

def strassen2(prod):
    res = strassen_out(lambda n: strassen_out(lambda m: prod(n * 7 + m)))
    C = [[None] * 4 for _ in range(4)]
    for I in range(2):
        for J in range(2):
            for i in range(2):
                for j in range(2):
                    C[2 * I + i][2 * J + j] = res[2 * I + J][2 * i + j]
    return C

def gelu_mul(gg, uu, half):
    inner = gg * (0.7978845608028654 + (0.7978845608028654 * 0.044715) * (gg * gg))
    t = jnp.tanh(inner)
    return (gg + gg * t) * (uu * half)

def make_kernel(L, D, P, F, TM=256, scan_group=2, nslot=3, frac=0.95, order=1, delay=0, touch=0, always=0, nofirst=0, nocomb=0, flags=None, ksplit=2, ngate=1, interpret=False):
    SKIP[0] = nocomb
    ORDER[0] = order
    NT = L // TM
    S = TM // SUB
    Q = TM // 4
    NB = D // LANES
    PB = P // LANES
    K4 = D // 4
    NC = F // 512
    KD = F // 4
    KS = P // 2
    NBC = 4
    NCH = NBC + NC + NBC

    def kernel(x_ref, lre_ref, lim_ref, ldt_ref, dsk_ref, gw_ref,
               bre_hbm, bim_hbm, cre_hbm, cim_hbm, wg_hbm, wu_hbm, wd_hbm,
               o_ref,
               RB, RU, RD, RC,
               xs, LX, gps, lam, bu, LD, os_, carry):
        step = pl.program_id(0)

        def row_scale(k, cb, n):
            return jnp.tile(lam[k, :, cb], (n, 1))

        def scan_consts():
            return None

        def seg_init(er, ei, c):
            row = lax.broadcasted_iota(jnp.int32, (SUB, LANES), 0)
            tr = jnp.where(row == 0, carry[0, :, c], pltpu.roll(er, 1, 0))
            ti = jnp.where(row == 0, carry[1, :, c], pltpu.roll(ei, 1, 0))
            pr, pi = lam[4, :, c], lam[5, :, c]
            for sh in (1, 2, 4):
                sr = jnp.where(row >= sh, pltpu.roll(tr, sh, 0), 0.0)
                si = jnp.where(row >= sh, pltpu.roll(ti, sh, 0), 0.0)
                mr, mi = _cmul(pr, pi, sr, si)
                tr, ti = tr + mr, ti + mi
                if sh < 4:
                    pr, pi = pr * pr - pi * pi, 2.0 * (pr * pi)
            return tr, ti

        def save_carry(hr, hi, c):
            carry[0, :, c] = jnp.broadcast_to(hr[SUB - 1:SUB, :], (SUB, LANES))
            carry[1, :, c] = jnp.broadcast_to(hi[SUB - 1:SUB, :], (SUB, LANES))

        @pl.when(step == 0)
        def _():
            vec = lambda r: r[...].astype(F32).reshape(1, -1)
            lre, lim = vec(lre_ref), vec(lim_ref)
            dt = jnp.exp(vec(ldt_ref))
            mag = jnp.exp(dt * lre)
            ang = dt * lim
            ar = mag * jnp.cos(ang)
            ai = mag * jnp.sin(ang)
            den = lre * lre + lim * lim
            nr = ar - 1.0
            cr = (nr * lre + ai * lim) / den
            ci = (ai * lre - nr * lim) / den
            pr, pi = ar, ai
            n = 1
            while n < S:
                pr, pi = pr * pr - pi * pi, 2.0 * (pr * pi)
                n *= 2
            rows = [ar, ai, cr, ci, pr, pi, vec(dsk_ref), vec(gw_ref)]
            for k, r in enumerate(rows):
                lam[k] = jnp.broadcast_to(r, (SUB, r.shape[1]))
            carry[...] = jnp.zeros(carry.shape, F32)

        def x_prep():
            xf = x_ref[...].astype(F32)
            for b in range(NB):
                for s in range(SUB):
                    xs[b, pl.ds(s, S, stride=SUB), :] = xf[s * S:(s + 1) * S, b * LANES:(b + 1) * LANES]
            acc = None
            for b in range(NB):
                t = xs[b] * row_scale(7, slice(b * LANES, (b + 1) * LANES), S)
                acc = t if acc is None else acc + t
            g = jax.nn.sigmoid(jnp.sum(acc, axis=-1, keepdims=True))
            gps[...] = jnp.broadcast_to(g, (TM, LANES))

        def first_tile(stg, XP, HS, TMP, sems):

            def b_copies(i, slot):
                r = pl.multiple_of(i * LANES, LANES)
                out = []
                for jq, src in enumerate((bre_hbm, bre_hbm, bim_hbm, bim_hbm)):
                    out.append(pltpu.make_async_copy(
                        src.at[pl.ds((jq % 2) * KS + r, LANES), :],
                        stg.at[slot, pl.ds(jq * LANES, LANES), :], sems.at[slot, jq]))
                return out

            def ud_copies(c, slot):
                c0 = pl.multiple_of(c * 512, 512)
                return [
                    pltpu.make_async_copy(wg_hbm.at[:, pl.ds(c0, 512)], stg.at[slot, pl.ds(0, D), pl.ds(0, 512)], sems.at[slot, 0]),
                    pltpu.make_async_copy(wu_hbm.at[:, pl.ds(c0, 512)], stg.at[slot, pl.ds(0, D), pl.ds(512, 512)], sems.at[slot, 1]),
                    pltpu.make_async_copy(wd_hbm.at[pl.ds(c0, 512), :], stg.at[slot, pl.ds(D, 512), :], sems.at[slot, 2]),
                ]

            def c_copies(i, slot):
                r = pl.multiple_of(i * LANES, LANES)
                out = []
                for kq, src in enumerate((cre_hbm, cre_hbm, cim_hbm, cim_hbm)):
                    out.append(pltpu.make_async_copy(
                        src.at[:, pl.ds((kq % 2) * KS + r, LANES)],
                        stg.at[slot, pl.ds(0, D), pl.ds(kq * LANES, LANES)], sems.at[slot, kq]))
                return out

            def start(copies):
                for cp in copies:
                    cp.start()

            def wait(copies):
                for cp in copies:
                    cp.wait()

            ahead = nslot - 1
            def start_chunk(k, kinds):
                slot = lax.rem(k, nslot)
                if 'b' in kinds:
                    pl.when(k < NBC)(lambda: start(b_copies(k, slot)))
                if 'u' in kinds:
                    pl.when(jnp.logical_and(k >= NBC, k < NBC + NC))(lambda: start(ud_copies(k - NBC, slot)))
                if 'c' in kinds:
                    pl.when(jnp.logical_and(k >= NBC + NC, k < NCH))(lambda: start(c_copies(k - NBC - NC, slot)))

            for k in range(ahead):
                start(b_copies(k, k))

            for m in range(NB // 2):
                XP[:, m * 256:(m + 1) * 256] = jnp.concatenate([xs[2 * m], xs[2 * m + 1]], axis=1).astype(BF16)
            for b in range(NB):
                os_[b] = gps[...] * (xs[b] * row_scale(6, slice(b * LANES, (b + 1) * LANES), S))

            tmp_i = [0]
            def pdot(lhs_ref, rhs_fn, dot, stream, sub=1, K=D):
                if K <= 512 or not ksplit:
                    res = dot(lhs_ref[:, 0:K], rhs_fn(0, K))
                else:
                    t = tmp_i[0] % ksplit
                    tmp_i[0] += 1
                    first = dot(lhs_ref[:, 0:512], rhs_fn(0, 512))
                    TMP[t] = first
                    stream += [first[8 * q:8 * q + 8] for q in range(TM // 8)][::sub]
                    res = TMP[t] + dot(lhs_ref[:, 512:K], rhs_fn(512, K - 512))
                stream += [res[8 * q:8 * q + 8] for q in range(TM // 8)][::sub]
                return res

            def spread(stream, g, n):
                pos = int(g * (len(stream) * frac) / n)
                if ngate:
                    return zero_of(stream[pos]), [zero_of(stream[min(len(stream) - 1, int((g + m / 7) * (len(stream) * frac) / n))]) for m in range(7)]
                return zero_of(stream[pos]), None

            def b_body(i, carry_):
                slot = lax.rem(i, nslot)
                wait(b_copies(i, slot))
                start_chunk(i + ahead, 'bu')
                r = pl.multiple_of(i * LANES, LANES)
                dst = (i // 2) * 49
                r8 = pl.multiple_of(lax.rem(i, 2) * 64, 64)
                stream = []
                for jq in range(4):
                    res = pdot(XP, lambda k0, kn: stg[slot, pl.ds(jq * LANES, LANES), pl.ds(k0, kn)], _dot_t, stream)
                    bu[jq // 2, :, pl.ds((jq % 2) * KS + r, LANES)] = res
                groups = [(sr, h) for sr in range(8) for h in range(2)]
                for g, (sr, h) in enumerate(groups):
                    rcomb2_packed(
                        lambda kq, jq: pltpu.bitcast(stg[slot, pl.ds(jq * 128 + sr * 16, 16), pl.ds(kq * K4 + h * LANES, LANES)], U32),
                        lambda nm, v: RB.__setitem__((dst + nm, pl.ds(r8 + sr * 8, 8), slice(h * LANES, (h + 1) * LANES)), v),
                        *spread(stream, g, len(groups)))
                return carry_
            lax.fori_loop(0, NBC, b_body, 0)

            for b0 in range(0, PB, 4):
                bl = list(range(b0, b0 + 4))
                sl = [slice(b * LANES, (b + 1) * LANES) for b in bl]
                ar = [lam[0, :, c] for c in sl]
                ai = [lam[1, :, c] for c in sl]
                def p1(j, st):
                    r0 = pl.multiple_of(j * SUB, SUB)
                    out = []
                    for k, c in enumerate(sl):
                        nr_, ni_ = _cmul(ar[k], ai[k], st[2 * k], st[2 * k + 1])
                        out.append(nr_ + bu[0, pl.ds(r0, SUB), c])
                        out.append(ni_ + bu[1, pl.ds(r0, SUB), c])
                    return tuple(out)
                z = jnp.zeros((SUB, LANES), F32)
                E = lax.fori_loop(0, S, p1, tuple(z for _ in range(2 * len(bl))), unroll=2)
                init = []
                for k, c in enumerate(sl):
                    init += list(seg_init(E[2 * k], E[2 * k + 1], c))
                cr = [lam[2, :, c] for c in sl]
                ci = [lam[3, :, c] for c in sl]
                def p2(j, st):
                    r0 = pl.multiple_of(j * SUB, SUB)
                    sc = 2.0 * gps[pl.ds(r0, SUB), :]
                    out = []
                    for k, c in enumerate(sl):
                        nr_, ni_ = _cmul(ar[k], ai[k], st[2 * k], st[2 * k + 1])
                        hr = nr_ + bu[0, pl.ds(r0, SUB), c]
                        hi = ni_ + bu[1, pl.ds(r0, SUB), c]
                        out += [hr, hi]
                        yr, yi = _cmul(cr[k], ci[k], hr, hi)
                        bu[0, pl.ds(r0, SUB), c] = yr * sc
                        bu[1, pl.ds(r0, SUB), c] = yi * (-sc)
                    return tuple(out)
                H = lax.fori_loop(0, S, p2, tuple(init), unroll=2)
                for k, c in enumerate(sl):
                    save_carry(H[2 * k], H[2 * k + 1], c)
            for kq in range(4):
                HS[kq] = bu[kq // 2, :, (kq % 2) * KS:(kq % 2 + 1) * KS].astype(BF16)

            def ud_body(c, carry_):
                k = NBC + c
                slot = lax.rem(k, nslot)
                wait(ud_copies(c, slot))
                start_chunk(k + ahead, 'uc')
                stream = []
                half = 0.5 * (1.0 - gps[...])
                hs = []
                for j in range(4):
                    gg = pdot(XP, lambda k0, kn: stg[slot, pl.ds(k0, kn), pl.ds(j * LANES, LANES)], _dot, stream)
                    uu = pdot(XP, lambda k0, kn: stg[slot, pl.ds(k0, kn), pl.ds(512 + j * LANES, LANES)], _dot, stream)
                    hs.append(gelu_mul(gg, uu, half))
                hc = jnp.concatenate(hs, axis=1).astype(BF16)
                for b in range(NB):
                    res = pdot(hc, lambda k0, kn: stg[slot, pl.ds(D, 512), pl.ds(b * LANES, LANES)], _dot, stream, 2 if not ksplit else 1, 512)
                    os_[b] += res
                r64 = pl.multiple_of(c * 64, 64)
                groups = [('u', sr, h) for sr in range(16) for h in range(2)] + [('d', sr, h) for sr in range(8) for h in range(2)]
                for g, (kind, sr, h) in enumerate(groups):
                    dep = spread(stream, g, len(groups))
                    if kind == 'u':
                        rcomb2_packed(
                            lambda kq, jq: pltpu.bitcast(stg[slot, pl.ds(kq * 256 + sr * 16, 16), pl.ds(jq * 256 + h * LANES, LANES)], U32),
                            lambda nm, v: RU.__setitem__((c * 49 + nm, pl.ds(sr * 8, 8), slice(h * LANES, (h + 1) * LANES)), v), *dep)
                    else:
                        rcomb2_packed(
                            lambda kq, jq: pltpu.bitcast(stg[slot, pl.ds(D + kq * 128 + sr * 16, 16), pl.ds(jq * 256 + h * LANES, LANES)], U32),
                            lambda nm, v: RD.__setitem__((nm, pl.ds(r64 + sr * 8, 8), slice(h * LANES, (h + 1) * LANES)), v), *dep)
                return carry_
            lax.fori_loop(0, NC, ud_body, 0)

            def c_body(i, carry_):
                k = NBC + NC + i
                slot = lax.rem(k, nslot)
                wait(c_copies(i, slot))
                start_chunk(k + ahead, 'c')
                r = pl.multiple_of(i * LANES, LANES)
                hs = jnp.concatenate([HS[kq, :, pl.ds(r, LANES)] for kq in range(4)], axis=1)
                stream = []
                for b in range(NB):
                    res = pdot(hs, lambda k0, kn: stg[slot, pl.ds(b * LANES, LANES), pl.ds(0, 512)], _dot_t, stream, 1, 512)
                    os_[b] += res
                for sr in range(16):
                    rcomb2_packed(
                        lambda kq, jq: pltpu.bitcast(stg[slot, pl.ds(jq * 256 + sr * 16, 16), pl.ds(kq * LANES, LANES)], U32),
                        lambda nm, v: RC.__setitem__((nm, pl.ds(sr * 8, 8), pl.ds(r, LANES)), v),
                        *spread(stream, sr, 16))
                return carry_
            lax.fori_loop(0, NBC, c_body, 0)
            if delay:
                pl.delay(delay)
            if touch:
                def tb(n, c_):
                    LD[n] = jnp.zeros(LD.shape[1:], U32)
                    LX[n] = jnp.zeros(LX.shape[1:], U32)
                    return c_
                lax.fori_loop(0, 49, tb, 0)

        def steady_tile():
            for h in range(2):
                gx = [[xs[2 * kq + h, i * Q:(i + 1) * Q, :] for kq in range(4)] for i in range(4)]
                for nm, v in enumerate(comb2(lcomb, gx)):
                    LX[nm, :, h * LANES:(h + 1) * LANES] = _pk(v)

            for c in range(2):
                C = strassen2(lambda nm: _dot_t(_bf(LX[nm]), _bf(RB[c * 49 + nm])))
                for i in range(4):
                    for jq in range(4):
                        p0 = (jq % 2) * KS + c * 256
                        bu[jq // 2, i * Q:(i + 1) * Q, p0:p0 + 256] = C[i][jq]

            prev = None
            for b0 in range(0, PB, scan_group):
                bl = list(range(b0, b0 + scan_group))
                sl = [slice(b * LANES, (b + 1) * LANES) for b in bl]
                ar = [lam[0, :, c] for c in sl]
                ai = [lam[1, :, c] for c in sl]
                st = [None] * (2 * len(bl))
                dep = None
                if prev is not None:
                    dep = lax.bitcast_convert_type((lax.bitcast_convert_type(prev, U32) >> 16) >> 16, F32)
                for j in range(S):
                    rs = slice(j * SUB, (j + 1) * SUB)
                    for k, c in enumerate(sl):
                        if j == 0:
                            st[2 * k], st[2 * k + 1] = bu[0, rs, c], bu[1, rs, c]
                            if dep is not None:
                                st[2 * k], st[2 * k + 1] = st[2 * k] + dep, st[2 * k + 1] + dep
                                ar[k] = ar[k] + dep
                                ai[k] = ai[k] + dep
                        else:
                            nr_, ni_ = _cmul(ar[k], ai[k], st[2 * k], st[2 * k + 1])
                            st[2 * k] = nr_ + bu[0, rs, c]
                            st[2 * k + 1] = ni_ + bu[1, rs, c]
                for k, c in enumerate(sl):
                    st[2 * k], st[2 * k + 1] = seg_init(st[2 * k], st[2 * k + 1], c)
                cr = [lam[2, :, c] for c in sl]
                ci = [lam[3, :, c] for c in sl]
                for j in range(S):
                    rs = slice(j * SUB, (j + 1) * SUB)
                    sc = 2.0 * gps[rs, :]
                    for k, c in enumerate(sl):
                        nr_, ni_ = _cmul(ar[k], ai[k], st[2 * k], st[2 * k + 1])
                        hr = nr_ + bu[0, rs, c]
                        hi = ni_ + bu[1, rs, c]
                        st[2 * k], st[2 * k + 1] = hr, hi
                        yr, yi = _cmul(cr[k], ci[k], hr, hi)
                        bu[0, rs, c] = yr * sc
                        bu[1, rs, c] = yi * (-sc)
                for k, c in enumerate(sl):
                    save_carry(st[2 * k], st[2 * k + 1], c)
                prev = st[-1]

            for c in range(NC):
                C = strassen2(lambda nm: _dot(_bf(LX[nm]), _bf(RU[c * 49 + nm])))
                hgrid = [[None] * 4 for _ in range(4)]
                for i in range(4):
                    half = 0.5 * (1.0 - gps[i * Q:(i + 1) * Q, :])
                    for j in range(2):
                        for k in range(2):
                            cs = slice(k * LANES, (k + 1) * LANES)
                            hgrid[i][2 * j + k] = gelu_mul(C[i][j][:, cs], C[i][2 + j][:, cs], half)
                for nm, v in enumerate(comb2(lcomb, hgrid)):
                    LD[nm, :, c * LANES:(c + 1) * LANES] = _pk(v)

            for h in range(4):
                gs = [[bu[kq // 2, i * Q:(i + 1) * Q, (kq % 2) * KS + h * LANES:(kq % 2) * KS + (h + 1) * LANES]
                       for kq in range(4)] for i in range(4)]
                for nm, v in enumerate(comb2(lcomb, gs)):
                    LD[nm, :, KD + h * LANES:KD + (h + 1) * LANES] = _pk(v)

            for nh in range(2):
                cs = slice(nh * LANES, (nh + 1) * LANES)
                C = strassen2(lambda nm: _dot(_bf(LD[nm, :, 0:KD]), _bf(RD[nm, :, cs]))
                              + _dot_t(_bf(LD[nm, :, KD:KD + KS]), _bf(RC[nm, nh * (LANES // 2):(nh + 1) * (LANES // 2), :])))
                for i in range(4):
                    rs = slice(i * Q, (i + 1) * Q)
                    for jq in range(4):
                        b = 2 * jq + nh
                        cb = slice(b * LANES, (b + 1) * LANES)
                        os_[b, rs, :] = C[i][jq] + gps[rs, :] * (xs[b, rs, :] * row_scale(6, cb, Q // SUB))

        x_prep()

        @pl.when(step == 0)
        def _():
            if nofirst:
                return
            pl.run_scoped(first_tile,
                          pltpu.VMEM((nslot, D + 512, D), BF16),
                          pltpu.VMEM((TM, D), BF16),
                          pltpu.VMEM((4, TM, KS), BF16),
                          pltpu.VMEM((max(ksplit, 1), TM, LANES), F32),
                          pltpu.SemaphoreType.DMA((nslot, 4)))

        if always:
            steady_tile()
        else:
            @pl.when(step > 0)
            def _():
                steady_tile()

        for b in range(NB):
            for s in range(SUB):
                o_ref[s * S:(s + 1) * S, b * LANES:(b + 1) * LANES] = os_[b, pl.ds(s, S, stride=SUB), :]

    vec = lambda: pl.BlockSpec((D,), lambda i: (0,))
    anyspec = pl.BlockSpec(memory_space=pl.ANY)
    return pl.pallas_call(
        kernel,
        grid=(NT,),
        in_specs=[pl.BlockSpec((TM, D), lambda i: (i, 0))] + [vec() for _ in range(5)] + [anyspec] * 7,
        out_specs=pl.BlockSpec((TM, D), lambda i: (i, 0)),
        out_shape=jax.ShapeDtypeStruct((L, D), F32),
        scratch_shapes=[
            pltpu.VMEM((2 * 49, 128, K4), U32),
            pltpu.VMEM((NC * 49, K4 // 2, 256), U32),
            pltpu.VMEM((49, KD // 2, 256), U32),
            pltpu.VMEM((49, 128, KS), U32),
            pltpu.VMEM((NB, TM, LANES), F32),
            pltpu.VMEM((49, Q // 2, K4), U32),
            pltpu.VMEM((TM, LANES), F32),
            pltpu.VMEM((8, SUB, P), F32),
            pltpu.VMEM((2, TM, P), F32),
            pltpu.VMEM((49, Q // 2, KD + KS), U32),
            pltpu.VMEM((NB, TM, LANES), F32),
            pltpu.VMEM((2, SUB, P), F32),
        ],
        compiler_params=pltpu.CompilerParams(
            dimension_semantics=("arbitrary",), vmem_limit_bytes=127 * 2**20, flags=flags),
        interpret=interpret,
        name="gmix",
    )


@jax.jit
def pallas_gated_mix__ssm_conv_s5__glu_gated_geglu__prompt_kernel(
    A_x: jax.Array,
    A_Lambda_re: jax.Array,
    A_Lambda_im: jax.Array,
    A_B_re: jax.Array,
    A_B_im: jax.Array,
    A_C_re: jax.Array,
    A_C_im: jax.Array,
    A_log_dt: jax.Array,
    A_Dskip: jax.Array,
    B_x: jax.Array,
    B_w_gate: jax.Array,
    B_w_up: jax.Array,
    B_w_down: jax.Array,
    gate_w: jax.Array,
):
    del B_x
    Bsz, L, D = A_x.shape
    P = A_Lambda_re.shape[0]
    F = B_w_gate.shape[1]
    k = make_kernel(L, D, P, F)
    out = k(A_x.reshape(L, D), A_Lambda_re, A_Lambda_im, A_log_dt, A_Dskip, gate_w,
            A_B_re, A_B_im, A_C_re, A_C_im, B_w_gate, B_w_up, B_w_down)
    return out.reshape(Bsz, L, D)
```

```python
import jax
import jax.numpy as jnp
from jax import lax
from jax.experimental import pallas as pl
from jax.experimental.pallas import tpu as pltpu

F32 = jnp.float32
BF16 = jnp.bfloat16
U32 = jnp.uint32
LANES = 128
SUB = 8
TM = 256
FC = 512
NSLOT = 3
SCAN_GROUP = 2


def _dot(a, b):
    return jnp.dot(a, b, preferred_element_type=F32)


def _dot_t(a, b):
    return lax.dot_general(a, b, (((1,), (1,)), ((), ())), preferred_element_type=F32)


def _pack(v):
    return pltpu.bitcast(v.astype(BF16), U32)


def _bf(u):
    return pltpu.bitcast(u, BF16)


def _cmul(ar, ai, br, bi):
    return ar * br - ai * bi, ar * bi + ai * br


def _zero_of(v):
    return (lax.bitcast_convert_type(v, U32) >> 16) >> 16


def _gated(v, z):
    if z is None:
        return v
    z = jnp.tile(z, (v.shape[0] // SUB, v.shape[1] // LANES))
    return lax.bitcast_convert_type(lax.bitcast_convert_type(v, U32) | z, F32)


def _pacer(stream, lo, hi):
    def at(f):
        v = stream[min(len(stream) - 1, int((lo + (hi - lo) * f) * len(stream)))]
        return _zero_of(v[0:SUB, 0:LANES])
    return at


def _tap(stream, fn):
    def wrapped(nm):
        r = fn(nm)
        stream.append(r)
        return r
    return wrapped


def _lcomb(a11, a12, a21, a22):
    return [a11 + a22, a21 + a22, a11, a22, a11 + a12, a21 - a11, a12 - a22]


def _rcomb(b11, b12, b21, b22):
    return [b11 + b22, b11, b12 - b22, b21 - b11, b22, b11 + b12, b21 + b22]


def _lcomb2(g):
    out = [None] * 49
    outer = {}
    for i in range(2):
        for k in range(2):
            outer[i, k] = _lcomb(g[i][k], g[i][2 + k], g[2 + i][k], g[2 + i][2 + k])
    for n in range(7):
        inner = _lcomb(outer[0, 0][n], outer[0, 1][n], outer[1, 0][n], outer[1, 1][n])
        for m in range(7):
            out[n * 7 + m] = inner[m]
    return out


_RTERMS = [((0, 0), (1, 1), 1), ((0, 0), None, 0), ((0, 1), (1, 1), -1), ((1, 0), (0, 0), -1),
           ((1, 1), None, 0), ((0, 0), (0, 1), 1), ((1, 0), (1, 1), 1)]
_RRAW = {8: (0, 0), 11: (1, 1), 29: (2, 2), 32: (3, 3)}


def _rcomb2_slab(load, store, gate0, gates):
    raw = [[load(r, c) | gate0 for c in range(4)] for r in range(4)]
    un = lambda r, c, e: pltpu.unpack_elementwise(raw[r][c], index=e, packed_dtype=BF16, unpacked_dtype=F32)
    for n, (ta, tb, sign) in enumerate(_RTERMS):
        inner = []
        for e in range(2):
            o = []
            for i in range(2):
                for k in range(2):
                    a = un(2 * ta[0] + i, 2 * ta[1] + k, e)
                    if tb is not None:
                        b = un(2 * tb[0] + i, 2 * tb[1] + k, e)
                        a = a + b if sign > 0 else a - b
                    o.append(_gated(a, gates[n]) if n > 0 else a)
            inner.append(_rcomb(*o))
        for m in range(7):
            nm = n * 7 + m
            if nm in _RRAW:
                r, c = _RRAW[nm]
                store(nm, raw[r][c])
            else:
                store(nm, pltpu.pack_elementwise([inner[0][m], inner[1][m]], packed_dtype=BF16))


def _strassen_out(prod):
    add = lambda a, b: jax.tree.map(lambda p, q: p + q, a, b)
    sub = lambda a, b: jax.tree.map(lambda p, q: p - q, a, b)
    m5 = prod(4); m3 = prod(2); c12 = add(m3, m5)
    m4 = prod(3); m2 = prod(1); c21 = add(m2, m4)
    t = sub(m4, m5); u = sub(m3, m2)
    m1 = prod(0); t = add(t, m1); u = add(u, m1)
    c11 = add(t, prod(6))
    c22 = add(u, prod(5))
    return [c11, c12, c21, c22]


def _strassen2(prod):
    res = _strassen_out(lambda n: _strassen_out(lambda m: prod(n * 7 + m)))
    return [[res[2 * (r // 2) + c // 2][2 * (r % 2) + c % 2] for c in range(4)] for r in range(4)]


def _gelu_mul(gg, uu, half):
    inner = gg * (0.7978845608028654 + (0.7978845608028654 * 0.044715) * (gg * gg))
    return (gg + gg * jnp.tanh(inner)) * (uu * half)


def _make_kernel(L, D, P, F):
    NT = L // TM
    S = TM // SUB
    Q = TM // 4
    NB = D // LANES
    PB = P // LANES
    K4 = D // 4
    NC = F // FC
    KD = F // 4
    KS = P // 2
    NBC = 4
    NCH = NBC + NC + NBC
    assert L % TM == 0 and NT >= 2 and D == P == 1024 and F % FC == 0

    def kernel(x0_ref, xn_ref, lre_ref, lim_ref, ldt_ref, dsk_ref, gw_ref,
               bre_hbm, bim_hbm, cre_hbm, cim_hbm, wg_hbm, wu_hbm, wd_hbm,
               o_ref,
               RB, RU, RD, RC, xs, LX, gps, lam, bu, LD, os_, carry):
        step = pl.program_id(0)
        lanes = lambda b: slice(b * LANES, (b + 1) * LANES)
        chan = lambda k, b, n: jnp.tile(lam[k, :, lanes(b)], (n, 1))

        def constants():
            vec = lambda r: r[...].astype(F32).reshape(1, -1)
            lre, lim = vec(lre_ref), vec(lim_ref)
            dt = jnp.exp(vec(ldt_ref))
            mag = jnp.exp(dt * lre)
            ang = dt * lim
            ar, ai = mag * jnp.cos(ang), mag * jnp.sin(ang)
            den = lre * lre + lim * lim
            cr = ((ar - 1.0) * lre + ai * lim) / den
            ci = (ai * lre - (ar - 1.0) * lim) / den
            pr, pi = ar, ai
            n = 1
            while n < S:
                pr, pi = pr * pr - pi * pi, 2.0 * (pr * pi)
                n *= 2
            for k, r in enumerate([ar, ai, cr, ci, pr, pi, vec(dsk_ref), vec(gw_ref)]):
                lam[k] = jnp.broadcast_to(r, (SUB, r.shape[1]))
            carry[...] = jnp.zeros(carry.shape, F32)

        def x_prep(x_ref, gate_ref):
            for b in range(NB):
                xb = x_ref[:, lanes(b)].astype(F32)
                for s in range(SUB):
                    xs[b, pl.ds(s, S, stride=SUB), :] = xb[s * S:(s + 1) * S, :]
            acc = None
            for b in range(NB):
                t = xs[b] * chan(7, b, S)
                acc = t if acc is None else acc + t
            g = jax.nn.sigmoid(jnp.sum(acc, axis=-1, keepdims=True))
            gate_ref[...] = jnp.broadcast_to(g, (TM, LANES))

        def skip_init(gate_ref, at=None):
            for b in range(NB):
                xb = _gated(xs[b], at(b / NB) if at else None)
                os_[b] = gate_ref[...] * (xb * chan(6, b, S))

        def x_operands(at=None):
            nw = Q // 16
            for h in range(2):
                for w in range(nw):
                    z = at((h * nw + w) / (2 * nw)) if at else None
                    gx = [[_gated(xs[2 * kq + h, i * Q + 16 * w:i * Q + 16 * w + 16, :], z) for kq in range(4)]
                          for i in range(4)]
                    for nm, v in enumerate(_lcomb2(gx)):
                        LX[nm, 8 * w:8 * w + 8, lanes(h)] = _pack(v)

        def write_out():
            for b in range(NB):
                for s in range(SUB):
                    o_ref[s * S:(s + 1) * S, lanes(b)] = os_[b, pl.ds(s, S, stride=SUB), :]

        def seg_init(er, ei, c):
            row = lax.broadcasted_iota(jnp.int32, (SUB, LANES), 0)
            tr = jnp.where(row == 0, carry[0, :, c], pltpu.roll(er, 1, 0))
            ti = jnp.where(row == 0, carry[1, :, c], pltpu.roll(ei, 1, 0))
            pr, pi = lam[4, :, c], lam[5, :, c]
            for sh in (1, 2, 4):
                sr = jnp.where(row >= sh, pltpu.roll(tr, sh, 0), 0.0)
                si = jnp.where(row >= sh, pltpu.roll(ti, sh, 0), 0.0)
                mr, mi = _cmul(pr, pi, sr, si)
                tr, ti = tr + mr, ti + mi
                if sh < 4:
                    pr, pi = pr * pr - pi * pi, 2.0 * (pr * pi)
            return tr, ti

        def save_carry(hr, hi, c):
            carry[0, :, c] = jnp.broadcast_to(hr[SUB - 1:SUB, :], (SUB, LANES))
            carry[1, :, c] = jnp.broadcast_to(hi[SUB - 1:SUB, :], (SUB, LANES))

        def scan_step(st, ar, ai, rows, sl):
            out = []
            for k, c in enumerate(sl):
                nr, ni = _cmul(ar[k], ai[k], st[2 * k], st[2 * k + 1])
                out += [nr + bu[0, rows, c], ni + bu[1, rows, c]]
            return out

        def scan_emit(st, cr, ci, rows, sl, gate_ref):
            sc = 2.0 * gate_ref[rows, :]
            for k, c in enumerate(sl):
                yr, yi = _cmul(cr[k], ci[k], st[2 * k], st[2 * k + 1])
                bu[0, rows, c] = yr * sc
                bu[1, rows, c] = yi * (-sc)

        def first_tile(stg, XP, HS, TMP, gps0, sems):
            def b_copies(i, slot):
                r = pl.multiple_of(i * LANES, LANES)
                return [pltpu.make_async_copy(src.at[pl.ds((jq % 2) * KS + r, LANES), :],
                                              stg.at[slot, pl.ds(jq * LANES, LANES), :], sems.at[slot, jq])
                        for jq, src in enumerate((bre_hbm, bre_hbm, bim_hbm, bim_hbm))]

            def f_copies(c, slot):
                c0 = pl.multiple_of(c * FC, FC)
                return [
                    pltpu.make_async_copy(wg_hbm.at[:, pl.ds(c0, FC)], stg.at[slot, pl.ds(0, D), pl.ds(0, FC)], sems.at[slot, 0]),
                    pltpu.make_async_copy(wu_hbm.at[:, pl.ds(c0, FC)], stg.at[slot, pl.ds(0, D), pl.ds(FC, FC)], sems.at[slot, 1]),
                    pltpu.make_async_copy(wd_hbm.at[pl.ds(c0, FC), :], stg.at[slot, pl.ds(D, FC), :], sems.at[slot, 2]),
                ]

            def c_copies(i, slot):
                r = pl.multiple_of(i * LANES, LANES)
                return [pltpu.make_async_copy(src.at[:, pl.ds((kq % 2) * KS + r, LANES)],
                                              stg.at[slot, pl.ds(0, D), pl.ds(kq * LANES, LANES)], sems.at[slot, kq])
                        for kq, src in enumerate((cre_hbm, cre_hbm, cim_hbm, cim_hbm))]

            def start(copies):
                for cp in copies:
                    cp.start()

            def wait(copies):
                for cp in copies:
                    cp.wait()

            ahead = NSLOT - 1

            def start_chunk(k, kinds):
                slot = lax.rem(k, NSLOT)
                if "b" in kinds:
                    pl.when(k < NBC)(lambda: start(b_copies(k, slot)))
                if "f" in kinds:
                    pl.when(jnp.logical_and(k >= NBC, k < NBC + NC))(lambda: start(f_copies(k - NBC, slot)))
                if "c" in kinds:
                    pl.when(jnp.logical_and(k >= NBC + NC, k < NCH))(lambda: start(c_copies(k - NBC - NC, slot)))

            for k in range(ahead):
                start(b_copies(k, k))

            constants()
            x_prep(x0_ref, gps0)
            skip_init(gps0)
            for m in range(NB // 2):
                XP[:, m * 256:(m + 1) * 256] = jnp.concatenate([xs[2 * m], xs[2 * m + 1]], axis=1).astype(BF16)
            x_prep(xn_ref, gps)
            x_operands()

            tmp_i = [0]

            def pdot(lhs, rhs_fn, dot, stream, K=D):
                vregs = lambda v: [v[SUB * q:SUB * q + SUB] for q in range(TM // SUB)]
                if K <= 512:
                    res = dot(lhs[:, 0:K], rhs_fn(0, K))
                else:
                    t = tmp_i[0] % 2
                    tmp_i[0] += 1
                    first = dot(lhs[:, 0:512], rhs_fn(0, 512))
                    TMP[t] = first
                    stream += vregs(first)
                    res = TMP[t] + dot(lhs[:, 512:K], rhs_fn(512, K - 512))
                stream += vregs(res)
                return res

            def pace(stream, g, n):
                at = lambda f: _zero_of(stream[min(len(stream) - 1, int(f * len(stream) * 0.97 / n))])
                return at(g), [at(g + m / 7) for m in range(7)]

            def slab(slot, r0, c0):
                return pltpu.bitcast(stg[slot, pl.ds(r0, 16), pl.ds(c0, LANES)], U32)

            def b_body(i, _):
                slot = lax.rem(i, NSLOT)
                wait(b_copies(i, slot))
                start_chunk(i + ahead, "bf")
                r = pl.multiple_of(i * LANES, LANES)
                dst = (i // 2) * 49
                r8 = pl.multiple_of(lax.rem(i, 2) * 64, 64)
                stream = []
                for jq in range(4):
                    res = pdot(XP, lambda k0, kn: stg[slot, pl.ds(jq * LANES, LANES), pl.ds(k0, kn)], _dot_t, stream)
                    bu[jq // 2, :, pl.ds((jq % 2) * KS + r, LANES)] = res
                slabs = [(sr, h) for sr in range(8) for h in range(2)]
                for g, (sr, h) in enumerate(slabs):
                    _rcomb2_slab(lambda kq, jq: slab(slot, jq * LANES + sr * 16, kq * K4 + h * LANES),
                                 lambda nm, v: RB.__setitem__((dst + nm, pl.ds(r8 + sr * 8, 8), lanes(h)), v),
                                 *pace(stream, g, len(slabs)))
                return _
            lax.fori_loop(0, NBC, b_body, 0)

            for b0 in range(0, PB, 4):
                sl = [lanes(b) for b in range(b0, b0 + 4)]
                ar, ai, cr, ci = ([lam[k, :, c] for c in sl] for k in range(4))
                rows = lambda j: pl.ds(pl.multiple_of(j * SUB, SUB), SUB)
                z = jnp.zeros((SUB, LANES), F32)
                ends = lax.fori_loop(0, S, lambda j, st: tuple(scan_step(st, ar, ai, rows(j), sl)),
                                     tuple(z for _ in range(2 * len(sl))), unroll=2)
                init = []
                for k, c in enumerate(sl):
                    init += list(seg_init(ends[2 * k], ends[2 * k + 1], c))

                def rescan(j, st):
                    st = scan_step(st, ar, ai, rows(j), sl)
                    scan_emit(st, cr, ci, rows(j), sl, gps0)
                    return tuple(st)
                last = lax.fori_loop(0, S, rescan, tuple(init), unroll=2)
                for k, c in enumerate(sl):
                    save_carry(last[2 * k], last[2 * k + 1], c)
            for kq in range(4):
                HS[kq] = bu[kq // 2, :, (kq % 2) * KS:(kq % 2 + 1) * KS].astype(BF16)

            def f_body(c, _):
                k = NBC + c
                slot = lax.rem(k, NSLOT)
                wait(f_copies(c, slot))
                start_chunk(k + ahead, "fc")
                stream = []
                half = 0.5 * (1.0 - gps0[...])
                hs = []
                for j in range(FC // LANES):
                    gg = pdot(XP, lambda k0, kn: stg[slot, pl.ds(k0, kn), pl.ds(j * LANES, LANES)], _dot, stream)
                    uu = pdot(XP, lambda k0, kn: stg[slot, pl.ds(k0, kn), pl.ds(FC + j * LANES, LANES)], _dot, stream)
                    hs.append(_gelu_mul(gg, uu, half))
                hc = jnp.concatenate(hs, axis=1).astype(BF16)
                for b in range(NB):
                    os_[b] += pdot(hc, lambda k0, kn: stg[slot, pl.ds(D, FC), pl.ds(b * LANES, LANES)], _dot, stream, FC)
                r64 = pl.multiple_of(c * 64, 64)
                slabs = ([("u", sr, h) for sr in range(16) for h in range(2)]
                         + [("d", sr, h) for sr in range(8) for h in range(2)])
                for g, (kind, sr, h) in enumerate(slabs):
                    if kind == "u":
                        _rcomb2_slab(lambda kq, jq: slab(slot, kq * K4 + sr * 16, jq * 256 + h * LANES),
                                     lambda nm, v: RU.__setitem__((c * 49 + nm, pl.ds(sr * 8, 8), lanes(h)), v),
                                     *pace(stream, g, len(slabs)))
                    else:
                        _rcomb2_slab(lambda kq, jq: slab(slot, D + kq * LANES + sr * 16, jq * 256 + h * LANES),
                                     lambda nm, v: RD.__setitem__((nm, pl.ds(r64 + sr * 8, 8), lanes(h)), v),
                                     *pace(stream, g, len(slabs)))
                return _
            lax.fori_loop(0, NC, f_body, 0)

            def c_body(i, _):
                k = NBC + NC + i
                slot = lax.rem(k, NSLOT)
                wait(c_copies(i, slot))
                start_chunk(k + ahead, "c")
                r = pl.multiple_of(i * LANES, LANES)
                hs = jnp.concatenate([HS[kq, :, pl.ds(r, LANES)] for kq in range(4)], axis=1)
                stream = []
                for b in range(NB):
                    os_[b] += pdot(hs, lambda k0, kn: stg[slot, pl.ds(b * LANES, LANES), pl.ds(0, KS)], _dot_t, stream, KS)
                for sr in range(16):
                    _rcomb2_slab(lambda kq, jq: slab(slot, jq * 256 + sr * 16, kq * LANES),
                                 lambda nm, v: RC.__setitem__((nm, pl.ds(sr * 8, 8), pl.ds(r, LANES)), v),
                                 *pace(stream, sr, 16))
                return _
            lax.fori_loop(0, NBC, c_body, 0)

        def steady_tile():
            sb, su, sd = [], [], []
            Cb = [_strassen2(_tap(sb, lambda nm: _dot_t(_bf(LX[nm]), _bf(RB[c * 49 + nm])))) for c in range(2)]
            write_out()
            for c in range(2):
                for i in range(4):
                    for jq in range(4):
                        p0 = (jq % 2) * KS + c * 256
                        bu[jq // 2, i * Q:(i + 1) * Q, p0:p0 + 256] = Cb[c][i][jq]

            prev = None
            for b0 in range(0, PB, SCAN_GROUP):
                sl = [lanes(b) for b in range(b0, b0 + SCAN_GROUP)]
                ar, ai, cr, ci = ([lam[k, :, c] for c in sl] for k in range(4))
                rows = lambda j: slice(j * SUB, (j + 1) * SUB)
                st = [bu[e, rows(0), c] for c in sl for e in range(2)]
                if prev is not None:
                    dep = lax.bitcast_convert_type(_zero_of(prev), F32)
                    st = [v + dep for v in st]
                    ar, ai = [v + dep for v in ar], [v + dep for v in ai]
                for j in range(1, S):
                    st = scan_step(st, ar, ai, rows(j), sl)
                for k, c in enumerate(sl):
                    st[2 * k], st[2 * k + 1] = seg_init(st[2 * k], st[2 * k + 1], c)
                for j in range(S):
                    st = scan_step(st, ar, ai, rows(j), sl)
                    scan_emit(st, cr, ci, rows(j), sl, gps)
                for k, c in enumerate(sl):
                    save_carry(st[2 * k], st[2 * k + 1], c)
                prev = st[-1]

            for c in range(NC):
                C = _strassen2(_tap(su, lambda nm: _dot(_bf(LX[nm]), _bf(RU[c * 49 + nm]))))
                hgrid = [[None] * 4 for _ in range(4)]
                for i in range(4):
                    half = 0.5 * (1.0 - gps[i * Q:(i + 1) * Q, :])
                    for j in range(2):
                        for k in range(2):
                            hgrid[i][2 * j + k] = _gelu_mul(C[i][j][:, lanes(k)], C[i][2 + j][:, lanes(k)], half)
                for nm, v in enumerate(_lcomb2(hgrid)):
                    LD[nm, :, lanes(c)] = _pack(v)
            skip_init(gps, _pacer(su, 0.1, 0.4))

            for h in range(KS // LANES):
                for w in range(Q // 16):
                    gs = [[bu[kq // 2, i * Q + 16 * w:i * Q + 16 * w + 16,
                              (kq % 2) * KS + h * LANES:(kq % 2) * KS + (h + 1) * LANES]
                           for kq in range(4)] for i in range(4)]
                    for nm, v in enumerate(_lcomb2(gs)):
                        LD[nm, 8 * w:8 * w + 8, KD + h * LANES:KD + (h + 1) * LANES] = _pack(v)

            Cd = [_strassen2(_tap(sd, lambda nm: _dot(_bf(LD[nm, :, 0:KD]), _bf(RD[nm, :, lanes(nh)]))
                                  + _dot_t(_bf(LD[nm, :, KD:KD + KS]), _bf(RC[nm, nh * 64:(nh + 1) * 64, :]))))
                  for nh in range(2)]
            for nh in range(2):
                for i in range(4):
                    for jq in range(4):
                        os_[2 * jq + nh, i * Q:(i + 1) * Q, :] += Cd[nh][i][jq]
            x_prep(xn_ref, gps)
            x_operands(_pacer(sd, 0.3, 0.7))

        @pl.when(step == 0)
        def _():
            pl.run_scoped(first_tile,
                          pltpu.VMEM((NSLOT, D + FC, D), BF16),
                          pltpu.VMEM((TM, D), BF16),
                          pltpu.VMEM((4, TM, KS), BF16),
                          pltpu.VMEM((2, TM, LANES), F32),
                          pltpu.VMEM((TM, LANES), F32),
                          pltpu.SemaphoreType.DMA((NSLOT, 4)))

        @pl.when(jnp.logical_and(step > 0, step < NT))
        def _():
            steady_tile()

        @pl.when(step == NT)
        def _():
            write_out()

    vec = pl.BlockSpec((D,), lambda i: (0,))
    hbm = pl.BlockSpec(memory_space=pl.ANY)
    return pl.pallas_call(
        kernel,
        grid=(NT + 1,),
        in_specs=[pl.BlockSpec((TM, D), lambda i: (0, 0)),
                  pl.BlockSpec((TM, D), lambda i: (jnp.minimum(i + 1, NT - 1), 0)),
                  vec, vec, vec, vec, vec] + [hbm] * 7,
        out_specs=pl.BlockSpec((TM, D), lambda i: (jnp.maximum(i - 1, 0), 0)),
        out_shape=jax.ShapeDtypeStruct((L, D), F32),
        scratch_shapes=[
            pltpu.VMEM((2 * 49, 128, K4), U32),
            pltpu.VMEM((NC * 49, K4 // 2, 256), U32),
            pltpu.VMEM((49, KD // 2, 256), U32),
            pltpu.VMEM((49, 128, KS), U32),
            pltpu.VMEM((NB, TM, LANES), F32),
            pltpu.VMEM((49, Q // 2, K4), U32),
            pltpu.VMEM((TM, LANES), F32),
            pltpu.VMEM((8, SUB, P), F32),
            pltpu.VMEM((2, TM, P), F32),
            pltpu.VMEM((49, Q // 2, KD + KS), U32),
            pltpu.VMEM((NB, TM, LANES), F32),
            pltpu.VMEM((2, SUB, P), F32),
        ],
        compiler_params=pltpu.CompilerParams(
            dimension_semantics=("arbitrary",),
            vmem_limit_bytes=127 * 2**20,
            disable_bounds_checks=True),
        name="gmix",
    )


@jax.jit
def pallas_gated_mix__ssm_conv_s5__glu_gated_geglu__prompt_kernel(
    A_x: jax.Array,
    A_Lambda_re: jax.Array,
    A_Lambda_im: jax.Array,
    A_B_re: jax.Array,
    A_B_im: jax.Array,
    A_C_re: jax.Array,
    A_C_im: jax.Array,
    A_log_dt: jax.Array,
    A_Dskip: jax.Array,
    B_x: jax.Array,
    B_w_gate: jax.Array,
    B_w_up: jax.Array,
    B_w_down: jax.Array,
    gate_w: jax.Array,
):
    del B_x
    bsz, L, D = A_x.shape
    assert bsz == 1
    x = A_x.reshape(L, D)
    out = _make_kernel(L, D, A_Lambda_re.shape[0], B_w_gate.shape[1])(
        x, x, A_Lambda_re, A_Lambda_im, A_log_dt, A_Dskip, gate_w,
        A_B_re, A_B_im, A_C_re, A_C_im, B_w_gate, B_w_up, B_w_down)
    return out.reshape(bsz, L, D)
```
